```python
import jax
import jax.numpy as jnp

def _softmax(x, axis=-1):
    return jax.nn.softmax(x, axis=axis)
def _gelu(x):
    return jax.nn.gelu(x, approximate=True)
def _silu(x):
    return jax.nn.silu(x)
def _sigmoid(x):
    return jax.nn.sigmoid(x)
def _layernorm(x, axis=-1, eps=1e-5):
    m = jnp.mean(x, axis=axis, keepdims=True)
    v = jnp.var(x, axis=axis, keepdims=True)
    return (x - m) / jnp.sqrt(v + eps)
def _scatter_add(tgt, idx, src, axis=0):
    return tgt.at[idx].add(src)
def _segment_sum(src, seg, n):
    return jax.ops.segment_sum(src, seg, n)
class _Rng:
    def __init__(self, key):
        self._k = key
    def _next(self):
        self._k, sub = jax.random.split(self._k)
        return sub
    def normal(self, shape):
        return jax.random.normal(self._next(), shape, dtype=jnp.bfloat16)
    def randint(self, lo, hi, shape):
        return jax.random.randint(self._next(), shape, lo, hi, dtype=jnp.int32)
    def uniform(self, shape, lo=0.0, hi=1.0):
        return jax.random.uniform(self._next(), shape, jnp.bfloat16, lo, hi)
    def permutation(self, n):
        return jax.random.permutation(self._next(), n)


kernel_name = 'concat_heads__mha_block_cached__gqa_block_cached__near_ridge'

def _fwd_setup_inputs():
    _rng = _Rng(jax.random.key(int.from_bytes(__import__("os").urandom(4), "little")))
    _w = (lambda a: (lambda t: t.astype(jnp.bfloat16) if jnp.issubdtype(t.dtype, jnp.floating) else t)(jnp.asarray(a)))
    def _A_setup():
        B, Sq, D = 8, 224, 448
        H, Sk, Dh = 16, 512, 256
        return {
            "x": _w((lambda *s: _rng.normal(s) * 0.05)(B, Sq, D)),
            "k_cache": _w((lambda *s: _rng.normal(s) * 0.05)(B, H, Sk, Dh)),
            "v_cache": _w((lambda *s: _rng.normal(s) * 0.05)(B, H, Sk, Dh)),
            "wq": _w((lambda *s: _rng.normal(s) * 0.05)(D, H * Dh) * (D ** -0.5)),
            "wo": _w((lambda *s: _rng.normal(s) * 0.05)(H * Dh, D) * ((H * Dh) ** -0.5)),
        }
    _A_in = _A_setup()

    def _B_setup():
        B, Sq, D = 8, 224, 448
        Hq, Hkv, Sk, Dh = 16, 16, 512, 256
        assert Hq % Hkv == 0, (Hq, Hkv)
        return {
            "x": _w((lambda *s: _rng.normal(s) * 0.05)(B, Sq, D)),
            "k_cache": _w((lambda *s: _rng.normal(s) * 0.05)(B, Hkv, Sk, Dh)),
            "v_cache": _w((lambda *s: _rng.normal(s) * 0.05)(B, Hkv, Sk, Dh)),
            "wq": _w((lambda *s: _rng.normal(s) * 0.05)(D, Hq * Dh) * (D ** -0.5)),
            "wo": _w((lambda *s: _rng.normal(s) * 0.05)(Hq * Dh, D) * ((Hq * Dh) ** -0.5)),
        }
    _B_in = _B_setup()

    return {
        "A_x": _A_in["x"],
        "A_k_cache": _A_in["k_cache"],
        "A_v_cache": _A_in["v_cache"],
        "A_wq": _A_in["wq"],
        "A_wo": _A_in["wo"],
        "B_x": _B_in["x"],
        "B_k_cache": _B_in["k_cache"],
        "B_v_cache": _B_in["v_cache"],
        "B_wq": _B_in["wq"],
        "B_wo": _B_in["wo"],
    }

def _fwd_reference(A_x, A_k_cache, A_v_cache, A_wq, A_wo, B_x, B_k_cache, B_v_cache, B_wq, B_wo):
    def _A_ref(x, k_cache, v_cache, wq, wo):
        B, Sq, D = x.shape
        H, Dh = 16, 256
        q = (lambda x, *d: x.transpose(*d))((x @ wq).reshape(B, Sq, H, Dh), 0, 2, 1, 3)
        scores = jnp.einsum("bhqd,bhkd->bhqk", q, k_cache) * (Dh ** -0.5)
        p = _softmax(scores, axis=-1)
        o = jnp.einsum("bhqk,bhkd->bhqd", p, v_cache)
        return (lambda x, *d: x.transpose(*d))(o, 0, 2, 1, 3).reshape(B, Sq, H * Dh) @ wo

    def _B_ref(x, k_cache, v_cache, wq, wo):
        B, Sq, D = x.shape
        Hq, Dh = 16, 256
        Hkv = k_cache.shape[1]
        rep = Hq // Hkv
        q = (lambda x, *d: x.transpose(*d))((x @ wq).reshape(B, Sq, Hq, Dh), 0, 2, 1, 3)
        k = jnp.repeat(k_cache, rep, axis=1)
        v = jnp.repeat(v_cache, rep, axis=1)
        scores = jnp.einsum("bhqd,bhkd->bhqk", q, k) * (Dh ** -0.5)
        p = _softmax(scores, axis=-1)
        o = jnp.einsum("bhqk,bhkd->bhqd", p, v)
        return (lambda x, *d: x.transpose(*d))(o, 0, 2, 1, 3).reshape(B, Sq, Hq * Dh) @ wo

    a = _A_ref(A_x, A_k_cache, A_v_cache, A_wq, A_wo)
    b = _B_ref(B_x, B_k_cache, B_v_cache, B_wq, B_wo)
    return jnp.concatenate([a, b], axis=-1)


def setup_inputs():
    _inp = _fwd_setup_inputs()
    _gk = jax.random.fold_in(jax.random.key(int.from_bytes(__import__("os").urandom(4), "little")), 2**31 - 1)
    _shapes = [[8, 224, 896]]
    _dtypes = ['bfloat16']
    _gks = jax.random.split(_gk, len(_shapes))
    _gs = [jax.random.normal(k, s, dtype=jnp.dtype(d)) * 0.05 for k, s, d in zip(_gks, _shapes, _dtypes)]
    _inp["grad_out"] = _gs[0]
    return _inp

def reference(A_x, A_k_cache, A_v_cache, A_wq, A_wo, B_x, B_k_cache, B_v_cache, B_wq, B_wo, grad_out):
    _const = dict()
    def _f(*_d):
        return _fwd_reference(**{'A_x': _d[0], 'A_k_cache': _d[1], 'A_v_cache': _d[2], 'A_wq': _d[3], 'A_wo': _d[4], 'B_x': _d[5], 'B_k_cache': _d[6], 'B_v_cache': _d[7], 'B_wq': _d[8], 'B_wo': _d[9], **_const})
    _out, _vjp = jax.vjp(_f, A_x, A_k_cache, A_v_cache, A_wq, A_wo, B_x, B_k_cache, B_v_cache, B_wq, B_wo)
    _grads = _vjp(grad_out)
    _out0 = jnp.asarray(_out)
    return (_out0, *[jnp.asarray(_g) for _g in _grads])
```

```python
import contextlib
import functools
import jax
import jax.numpy as jnp
from jax import lax
from jax.experimental import pallas as pl
from jax.experimental.pallas import tpu as pltpu

NB, SQ, D, H, SK, DH = 8, 224, 448, 16, 512, 256
HQ, HD, HK, HH = SQ // 2, D // 2, SK // 2, DH // 2
NR = NB * HQ
R = 7
DP = 512
SCALE = DH ** -0.5
BF, F32, U32 = jnp.bfloat16, jnp.float32, jnp.uint32
NN = (((1,), (0,)), ((), ()))
NT = (((1,), (1,)), ((), ()))
TN = (((0,), (0,)), ((), ()))


def _dot(a, b, dn):
    return lax.dot_general(a, b, dn, preferred_element_type=F32)


def forms_u(a11, a12, a21, a22):
    return [a11 + a22, a21 + a22, a11, a22, a11 + a12, a21 - a11, a12 - a22]


def forms_v(b11, b12, b21, b22):
    return [b11 + b22, b11, b12 - b22, b21 - b11, b22, b11 + b12, b21 + b22]


def forms_w(c11, c12, c21, c22):
    return [c11 + c22, c21 - c22, c12 + c22, c11 + c21, c12 - c11, c22, c11]


def comb_w(m):
    return (m[0] + m[3] - m[4] + m[6], m[2] + m[4], m[1] + m[3], m[0] - m[1] + m[2] + m[5])


def comb_u(d):
    return (d[0] + d[2] + d[4] - d[5], d[4] + d[6], d[1] + d[5], d[0] + d[1] + d[3] - d[6])


def comb_v(d):
    return (d[0] + d[1] - d[3] + d[5], d[2] + d[5], d[3] + d[6], d[0] - d[2] + d[4] + d[6])


def _pk(x):
    return pltpu.bitcast(x.astype(BF), U32)


def _un(x):
    return pltpu.bitcast(x, BF)


def _bf(xs):
    return [x.astype(BF) for x in xs]


COST = dict(P=(56, 14, 14, 30), S=(56, 28, 0, 23), Y=(56, 14, 14, 30), Z=(64, 32, 0, 37), A=(56, 28, 28, 50),
            PC=(0, 7, 33, 14), YC=(0, 7, 33, 14), KV=(0, 5, 23, 8), SM=(0, 40, 300, 70), ZC=(0, 8, 24, 14),
            WF=(0, 110, 350, 120), F=(0, 130, 400, 200))


def mix(*lists):
    items = [((i + 0.5) / len(l), k, t) for k, l in enumerate(lists) for i, t in enumerate(l)]
    return [t for _, _, t in sorted(items, key=lambda z: z[:2])]


def plan(cfg):
    ok = lambda b: 0 <= b < NB
    ro = dict(P=(0, 1, 3, 5, 2, 6, 4), S=(0, 3, 4, 6, 1, 2, 5), Y=(0, 2, 4, 5, 1, 3, 6), Z=(0, 1, 3, 5, 2, 6, 4))
    G = lambda n, b: [(n, b, h, r) for h in range(2) for r in ro[n]] if ok(b) else []
    A = lambda tl: [('A', tl, h, r) for h in range(2) for r in range(R)] if 0 <= tl < 7 else []
    W = lambda lo, hi: [('W', lo, hi, h, r) for h in range(2) for r in range(R)]
    pair = lambda l: [l[i:i + 2] for i in range(0, len(l), 2)]
    pmix = lambda *ls: [t for p in mix(*[pair(l) for l in ls if l]) for t in p]
    o = cfg.get('order', 0)
    mm = G('P', 0) + G('P', 1)
    for b in range(NB + 1):
        if o == 0:
            mm += G('S', b) + G('P', b + 2) + G('Z', b - 1) + G('Y', b - 1)
        elif o == 1:
            mm += G('S', b) + G('P', b + 2) + G('Z', b - 1) + A(b - 4) + G('Y', b - 1)
        elif o == 2:
            mm += pmix(G('S', b), G('P', b + 2)) + pmix(G('Z', b - 1), G('Y', b - 1), A(b - 4))
        elif o == 3:
            mm += pmix(G('S', b), G('P', b + 2), A(b - 4)) + pmix(G('Y', b - 1), G('Z', b - 1))
        elif o == 5:
            z, y = G('Z', b - 1), G('Y', b - 1)
            mm += pmix(G('S', b), G('P', b + 2), A(b - 4)) + z[:8] + y[:6] + z[8:] + y[6:]
        elif o == 6:
            z, y = G('Z', b - 1), G('Y', b - 1)
            mm += pmix(G('S', b), G('P', b + 2), A(b - 4)) + z + y
        elif o == 7:
            sp_ = pmix(G('S', b), G('P', b + 2), A(b - 4))
            k = (len(sp_) // 4) * 2
            z, y = G('Z', b - 1), G('Y', b - 1)
            mm += sp_[:k] + z[:8] + y[:6] + sp_[k:] + z[8:] + y[6:]
        elif o == 4:
            mm += G('S', b) + G('P', b + 2) + A(b - 4) + G('Y', b - 1) + G('Z', b - 1)
    if o == 0:
        mm += [t for tl in range(7) for t in A(tl)] + W(0, 7)
    else:
        mm += A(5) + A(6) + W(0, 7)
    dur = lambda t: 56 * (t[2] - t[1]) if t[0] == 'W' else COST[t[0]][0]
    start, tt = {}, 0
    for t in mm:
        start[t] = tt
        tt += dur(t)
    total = tt
    end = lambda ts: max(start[t] + dur(t) for t in ts)
    beg = lambda ts: min([start[t] for t in ts] + [total])
    sel = lambda n, *k: [t for t in mm if t[0] == n and t[1:1 + len(k)] == k]
    lat, lead = cfg.get('lat', 56), cfg.get('lead', 112)
    vec = []
    for b in range(NB):
        for h in range(2):
            for c in range(7):
                vec.append((('PC', b, h, c), max(end(sel('P', b, h)), end(sel('Z', b - 3)) if b >= 3 else 0),
                            min(beg(sel('S', b, h)), beg(sel('P', b + 2, h)))))
                tl = (b * 112 + c * 16) // 128
                vec.append((('YC', b, h, c), end(sel('Y', b, h)), min(beg(sel('A', tl, h) + sel('W')), beg(sel('Y', b + 2, h)))))
            for c in range(16):
                vec.append((('KV', b, h, c), max(end(sel('Y', b - 3)) if b >= 3 else -lat, beg(sel('S', b)) - cfg.get('kvw', 3000)), beg(sel('S', b, h))))
                if not cfg.get('zm'): vec.append((('ZC', b, h, c), end(sel('Z', b, h)), min(beg(sel('Z', b + 2, h)), end(sel('Z', b, h)) + cfg.get('zcw', 2000))))
        for c in range(7):
            vec.append((('SM', b, c), max(end(sel('S', b)), end(sel('Z', b - 2) + sel('Y', b - 2)) if b >= 2 else 0),
                        min(beg(sel('Y', b) + sel('Z', b)), beg(sel('S', b + 2)))))
    for h in range(2):
        vec.append((('WF', h), beg(sel('W')), total))
        vec.append((('F', h), end(sel('W', 0, 7, h)), total + 1000))
    vec.sort(key=lambda v: v[2])
    fs, fv = cfg.get('fs', 0.6), cfg.get('fv', 0.5)
    out, st, va = [], 0.0, 0.0
    for i, t in enumerate(mm):
        now = start[t]
        k = 0
        while k < len(vec):
            v, rdy, dl = vec[k]
            c = COST[v[0]]
            forced = dl <= now + lead and rdy <= now
            if forced or (rdy + lat <= now and st + c[1] / fs <= now and va + c[2] / (4 * fv) <= now):
                out.append(v)
                st = max(st, now - 200) + c[1] / fs
                va = max(va, now - 200) + c[2] / (4 * fv)
                vec.pop(k)
            else:
                assert dl > now, (v, rdy, dl, now)
                if rdy + lat <= now and dl > now + lead:
                    break
                k += 1
        out.append(t)
        if cfg.get('zm') and t[0] == 'Z' and t[3] in (5, 4):
            out.append(('ZP', t[1], t[2], 0 if t[3] == 5 else 1))
        c = (0, 28, 28 * (t[2] - t[1]), 0) if t[0] == 'W' else COST[t[0]]
        st = max(st, now - 200) + c[1] / fs
        va = max(va, now - 200) + c[2] / (4 * fv)
    out += [v for v, _, _ in vec]
    return out


def _kernel(ax, ak, av, awq, awo, bx, bk, bv, bwq, bwo, g_hbm,
            out_hbm, dax, dak, dav, dawq, dawo, dbx, dbk, dbv, dbwq, dbwo,
            xin, gin, dxst, ost, tt, tail, xw, xwt, acc, vy, wu, pp, uf, vf, sp, wf, yp, zp, du,
            kbuf, vbuf, dkbuf, dvbuf, wqbuf, wobuf, dwqbuf, dwobuf,
            sem_in, sem_out, sem_misc, *, cfg):
    nt = 2 * H
    sc = jax.named_scope if cfg.get('prof') else (lambda n: contextlib.nullcontext())

    def in_copies(k_hbm, v_hbm, wq_hbm, wo_hbm, h, s):
        col = pl.ds(h * DH if isinstance(h, int) else pl.multiple_of(h * DH, DH), DH)
        if wq_hbm is not None:
            return [
                pltpu.make_async_copy(wq_hbm.at[:, col], wqbuf.at[s], sem_in.at[0, s]),
                pltpu.make_async_copy(wo_hbm.at[:, col], wobuf.at[s], sem_in.at[1, s]),
            ]
        if cfg.get('noin'):
            return []
        return [
            pltpu.make_async_copy(k_hbm.at[:, h], kbuf.at[s], sem_in.at[2, s]),
            pltpu.make_async_copy(v_hbm.at[:, h], vbuf.at[s], sem_in.at[3, s]),
        ]

    def out_copies(dk_hbm, dv_hbm, dwq_hbm, dwo_hbm, h, s):
        col = pl.ds(h * DH if isinstance(h, int) else pl.multiple_of(h * DH, DH), DH)
        if cfg.get('noout'):
            return []
        if cfg.get('dsplit'):
            kv_ = [pltpu.make_async_copy(buf.at[s, k], hbm.at[:, h, :, pl.ds(k * HH, HH)], sem_out.at[i, s])
                   for i, (buf, hbm) in enumerate(((dkbuf, dk_hbm), (dvbuf, dv_hbm))) for k in range(2)]
        else:
            kv_ = [pltpu.make_async_copy(dkbuf.at[s], dk_hbm.at[:, h], sem_out.at[0, s]),
                   pltpu.make_async_copy(dvbuf.at[s], dv_hbm.at[:, h], sem_out.at[1, s])]
        return kv_ + [
            pltpu.make_async_copy(dwqbuf.at[s], dwq_hbm.at[:, col], sem_out.at[2, s]),
            pltpu.make_async_copy(dwobuf.at[s], dwo_hbm.at[:, col], sem_out.at[3, s]),
        ]

    def start_in(tt, s, w):
        @pl.when(tt < H)
        def _():
            for c in in_copies(ak, av, awq if w else None, awo, tt, s):
                c.start()

        @pl.when(tt >= H)
        def _():
            for c in in_copies(bk, bv, bwq if w else None, bwo, jnp.minimum(tt - H, H - 1), s):
                c.start()

    def by_half(hbm, vm, sem, lanes=None, vlanes=None, out=False):
        cs = []
        for b in range(NB):
            for j in range(2):
                h_ = hbm.at[b, pl.ds(j * HQ, HQ)] if lanes is None else hbm.at[b, pl.ds(j * HQ, HQ), lanes]
                v_ = vm.at[j, pl.ds(b * HQ, HQ)] if vlanes is None else vm.at[j, pl.ds(b * HQ, HQ), vlanes]
                cs.append(pltpu.make_async_copy(v_, h_, sem) if out else pltpu.make_async_copy(h_, v_, sem))
        return cs

    x_in = [by_half(x_, xin, sem_misc.at[0]) for x_ in (ax, bx)]
    g_in = [by_half(g_hbm, gin, sem_misc.at[1], pl.ds(lo, DP)) for lo in (0, 2 * D - DP)]
    dx_out = [by_half(x_, dxst, sem_misc.at[2], out=True) for x_ in (dax, dbx)]
    o_out = [by_half(out_hbm, ost, sem_misc.at[3], pl.ds(0, 2 * D - DP), pl.ds(0, 2 * D - DP), out=True),
             by_half(out_hbm, ost, sem_misc.at[3], pl.ds(2 * D - DP, DP), out=True)]

    def weight_forms(s, half):
        w = wqbuf[s].astype(F32) * SCALE if half == 0 else wobuf[s].astype(F32)
        fs = forms_u(w[:HD, :HH], w[:HD, HH:], w[HD:, :HH], w[HD:, HH:])
        for r in range(R):
            wu[s, half, r, :HD, :] = fs[r].astype(BF)

    def head(t, carry):
        slot = t % 2

        @pl.when(t + 1 < nt)
        def _():
            start_in(t + 1, 1 - slot, False)
            start_in(t + 2, slot, True)

        with sc('headwait'):
            for c in in_copies(ak, av, None, None, 0, slot) + in_copies(ak, av, awq, awo, 0, 1 - slot):
                c.wait()

            @pl.when(t >= 2)
            def _():
                for c in out_copies(dak, dav, dawq, dawo, 0, slot):
                    c.wait()

        opq = cfg.get('opq', '')
        z_st, z_ld = jnp.minimum(t, 0), jnp.minimum(t + 1, 0)

        def rows(c, n=16):
            return slice(c * n, (c + 1) * n)

        def st32(name, ref, half, r, val):
            ref[half + (z_st if name in opq else 0), r] = val

        def ld32(name, ref, half, r, rr):
            return ref[half + (z_ld if name in opq else 0), r, rr, :]

        def st16(name, ref, half, r, rr, val):
            hh = half + (z_st if name in opq else 0)
            if len(ref.shape) == 4:
                ref[hh, r, rr, :] = val.astype(BF)
            else:
                for n in range(ref.shape[2]):
                    ref[hh, r, n, rr, :] = val[:, n * 128:(n + 1) * 128].astype(BF)

        def ld16(name, ref, half, r, rr=slice(None), nn=None):
            hh = half + (z_ld if name in opq else 0)
            if len(ref.shape) == 4:
                return _un(ref.bitcast(U32)[hh, r, rr, :])
            nn = range(ref.shape[2]) if nn is None else nn
            return jnp.concatenate([_un(ref.bitcast(U32)[hh, r, n, rr, :]) for n in nn], axis=1)

        def p_mm(b, half, r):
            st32('p', pp[b % 2], half, r, _dot(ld16('-', xwt, half, r, rows(b, HQ // 2)), _un(wu.bitcast(U32)[slot, half, r]), NN))

        def p_comb(b, half, c):
            t11, t12, t21, t22 = comb_v([ld32('p', pp[b % 2], half, r, rows(c)) for r in range(R)])
            for r, f in enumerate(forms_u(t11, t21, t12, t22)):
                st16('u', uf[b % 3], half, r, rows(c), f)

        def kv_blk(b, half, j, k, c=None):
            buf = (kbuf, vbuf)[half]
            rr = slice(j * HK, (j + 1) * HK) if c is None else slice(j * HK + c * 16, j * HK + c * 16 + 16)
            return buf[slot, b, rr, k * HH:(k + 1) * HH]

        def kv_forms(b, half, c):
            raw = [kv_blk(b, half, j, k, c).astype(F32) for (j, k) in ((0, 0), (1, 0), (0, 1), (1, 1))]
            for r, f in enumerate(forms_v(*raw)):
                if r not in (1, 4):
                    st16('v', vf[b % 3], half, r, rows(c), f)

        def v_form(b, half, r):
            if r == 1:
                return kv_blk(b, half, 0, 0)
            if r == 4:
                return kv_blk(b, half, 1, 1)
            return ld16('v', vf[b % 3], half, r)

        def s_mm(b, half, r):
            st32('s', sp[b % 2], half, r, _dot(ld16('u', uf[b % 3], half, r), v_form(b, half, r), NT))

        def softmax(b, c):
            cat = lambda x, i: jnp.concatenate([x[0][i], x[1][i]], axis=0)
            ps = []
            for c8 in (2 * c, 2 * c + 1):
                s11, s12, s21, s22 = comb_w([ld32('s', sp[b % 2], 0, r, rows(c8, 8)) for r in range(R)])
                p4 = []
                for (sa, sb) in ((s11, s12), (s21, s22)):
                    m = jnp.max(jnp.maximum(sa, sb), axis=-1, keepdims=True)
                    ea, eb = jnp.exp(sa - m), jnp.exp(sb - m)
                    l = jnp.sum(ea + eb, axis=-1, keepdims=True)
                    inv = pl.reciprocal(l, approx=True)
                    inv = inv * (2.0 - l * inv)
                    p4 += [ea * inv, eb * inv]
                ps.append(p4)
            for r, f in enumerate(forms_w(*[cat(ps, i) for i in range(4)])):
                st16('w', wf[b % 2], 1, r, rows(c), f)
            dss = []
            for p4, c8 in zip(ps, (2 * c, 2 * c + 1)):
                d4 = comb_w([ld32('s', sp[b % 2], 1, r, rows(c8, 8)) for r in range(R)])
                ds4 = []
                for i in (0, 2):
                    delta = jnp.sum(p4[i] * d4[i] + p4[i + 1] * d4[i + 1], axis=-1, keepdims=True)
                    ds4 += [p4[i] * (d4[i] - delta), p4[i + 1] * (d4[i + 1] - delta)]
                dss.append(ds4)
            for r, f in enumerate(forms_w(*[cat(dss, i) for i in range(4)])):
                st16('w', wf[b % 2], 0, r, rows(c), f)

        def y_mm(b, half, r):
            st32('y', yp[b % 2], half, r, _dot(ld16('w', wf[b % 2], half, r), v_form(b, half, r), NN))

        def y_comb(b, half, c):
            y11, y12, y21, y22 = comb_u([ld32('y', yp[b % 2], half, r, rows(c)) for r in range(R)])
            for r, f in enumerate(forms_v(y11, y21, y12, y22)):
                st16('x', vy, half, r, rows(b * 7 + c), f)

        zv = {}
        zt = cfg.get('zt', 0)

        def z_put(b, half, k, j, rr, val):
            buf = (dkbuf, dvbuf)[half]
            rr = pl.ds(j * HK + rr[0], rr[1])
            if cfg.get('dsplit'):
                buf[slot, k, b, rr, :] = val
            else:
                buf[slot, b, rr, k * HH:(k + 1) * HH] = val

        def z_mm(b, half, r):
            w_, u_ = ld16('w', wf[b % 2], half, r), ld16('u', uf[b % 3], half, r)
            zv[b, half, r] = _dot(u_, w_, TN) if zt else _dot(w_, u_, TN)

        def z_comb(b, half, c):
            z = comb_v([zv[b, half, r][rows(c)] for r in range(R)])
            for (k, j), zz in zip(((0, 0), (0, 1), (1, 0), (1, 1)), z):
                z_put(b, half, k, j, (c * 16, 16), zz.astype(BF))

        def z_part(b, half, part):
            d = lambda r: zv[b, half, r]
            fin = (lambda x: x.astype(BF).T) if zt else (lambda x: x.astype(BF))
            if part == 0:
                z_put(b, half, 0, 0, (0, HK), fin(d(0) + d(1) - d(3) + d(5)))
            else:
                z_put(b, half, 0, 1, (0, HK), fin(d(2) + d(5)))
                z_put(b, half, 1, 0, (0, HK), fin(d(3) + d(6)))
                z_put(b, half, 1, 1, (0, HK), fin(d(0) - d(2) + d(6) + d(4)))

        def acc_mm(tl, half, r):
            acc[half, r, :, rows(tl, 128)] += _dot(_un(wu.bitcast(U32)[slot, half, r, :HD // 2, :]), ld16('x', vy, half, r, rows(tl, 64)), NT)

        def dw_mm(lo, hi, half, r):
            d = _dot(ld16('-', xw, half, r, nn=range(lo, hi)), ld16('x', vy, half, r, slice(lo * 64, hi * 64)), NN)
            if lo == 0:
                du[half, r] = d
            else:
                du[half, r] += d

        def post_fin(s, half):
            a11, a12, a21, a22 = comb_u([du[half, r] for r in range(R)])
            dw = jnp.concatenate([jnp.concatenate([a11, a12], axis=1),
                                  jnp.concatenate([a21, a22], axis=1)], axis=0)
            if half == 0:
                dwqbuf[s] = (dw * SCALE).astype(BF)
            else:
                dwobuf[s] = dw.astype(BF)

        fns = dict(P=p_mm, PC=p_comb, KV=kv_forms, S=s_mm, SM=softmax, Y=y_mm, YC=y_comb, Z=z_mm, ZC=z_comb,
                   ZP=z_part, A=acc_mm, W=dw_mm, WF=lambda half: weight_forms(1 - slot, half),
                   F=lambda half: post_fin(slot, half))

        def body(_, cc):
            for task in plan(cfg):
                fns[task[0]](*task[1:])
            return cc

        with sc('body'):
            if cfg.get('rep', 1) == 1:
                body(0, 0)
            else:
                lax.fori_loop(0, cfg['rep'], body, 0)

        @pl.when(t < H)
        def _():
            for c in out_copies(dak, dav, dawq, dawo, t, slot):
                c.start()

        @pl.when(t >= H)
        def _():
            for c in out_copies(dbk, dbv, dbwq, dbwo, jnp.maximum(t - H, 0), slot):
                c.start()
        return carry

    def branch(br, carry):
        with sc('xwait'):
            for c in x_in[0] + g_in[0]:
                c.wait()
        off = pl.multiple_of(br * (DP - D), DP - D)

        def tile(n, carry):
            rr = pl.ds(pl.multiple_of(n * 128, 128), 128)
            for half in range(2):
                if half == 0:
                    ts = [xin[j, rr, :].T for j in range(2)]
                else:
                    for j in range(2):
                        tt[j, :DP, :] = gin[j, rr, :].T
                    ts = [tt[j, pl.ds(off, D), :] for j in range(2)]
                ts = [x_.astype(F32) for x_ in ts]
                fs = forms_w(ts[0][:HD], ts[1][:HD], ts[0][HD:], ts[1][HD:])
                for r in range(R):
                    f = fs[r].astype(BF)
                    xw[half, r, n] = f
                    ft = jnp.concatenate([f, jnp.zeros((DH - HD, 128), BF)], axis=0).T
                    for m in range(2):
                        xwt[half, r, m, rr, :] = ft[:, m * 128:(m + 1) * 128]
            return carry
        with sc('tiles'):
            lax.fori_loop(0, NR // 128, tile, 0)

        @pl.when(br == 0)
        def _():
            for c in x_in[1] + g_in[1]:
                c.start()

        with sc('heads'):
            lax.fori_loop(br * H, (br + 1) * H, head, 0)

        @pl.when(br == 1)
        def _():
            for c in dx_out[0] + o_out[0]:
                c.wait()
        off = pl.multiple_of((1 - br) * (DP - D), DP - D)

        def tile(n, carry):
            cc = pl.ds(pl.multiple_of(n * 128, 128), 128)
            for half in range(2):
                c11, c12, c21, c22 = comb_w([acc[half, r, :, cc] for r in range(R)])
                for r in range(R):
                    acc[half, r, :, cc] = jnp.zeros((HD, 128), F32)
                for j, (top, bot) in enumerate(((c11, c21), (c12, c22))):
                    y = jnp.concatenate([top, bot], axis=0).astype(BF)
                    if half == 0:
                        y = jnp.concatenate([y, jnp.zeros((DP - D, 128), BF)], axis=0)
                        dxst[j, cc, :] = y.T[:, :D]
                    else:
                        tt[j, :DP - D, :] = tail[j, n]
                        tt[j, DP - D:DP, :] = y
                        tt[j, DP:, :] = jnp.zeros((DP - D, 128), BF)
                        tail[j, n] = y[2 * D - DP:]
                        ost[j, cc, :] = tt[j, pl.ds(off, DP), :].T
            return carry
        with sc('tiles'):
            lax.fori_loop(0, NR // 128, tile, 0)

        @pl.when(br == 0)
        def _():
            for c in dx_out[0] + o_out[0]:
                c.start()
        return carry

    with sc('startup'):
        for c in x_in[0] + g_in[0]:
            c.start()
        for c in in_copies(ak, av, awq, awo, 0, 0) + in_copies(ak, av, None, None, 0, 0) + in_copies(ak, av, awq, awo, 1, 1):
            c.start()
        wu[...] = jnp.zeros(wu.shape, BF)
        tail[...] = jnp.zeros(tail.shape, BF)

        def zero(i, carry):
            acc[i // R, i % R] = jnp.zeros((HD, NR), F32)
            return carry
        lax.fori_loop(0, 2 * R, zero, 0)
        for c in in_copies(ak, av, awq, awo, 0, 0):
            c.wait()
        for half in range(2):
            weight_forms(0, half)
    lax.fori_loop(0, 2, branch, 0)
    with sc('drain'):
        for c in dx_out[1] + o_out[1]:
            c.start()
        for c in out_copies(dak, dav, dawq, dawo, 0, 0) + out_copies(dak, dav, dawq, dawo, 0, 1) + dx_out[1] + o_out[1]:
            c.wait()


def make(flags=None, lp=1, **cfg):
    if lp:
        flags = dict(flags or {}, XLA_TPU_FORCE_LP_LLO_SCHEDULER=True)
    @jax.jit
    def fn(A_x, A_k_cache, A_v_cache, A_wq, A_wo, B_x, B_k_cache, B_v_cache, B_wq, B_wo, grad_out):
        sds = lambda a: jax.ShapeDtypeStruct(a.shape, BF)
        ins = (A_x, A_k_cache, A_v_cache, A_wq, A_wo.T, B_x, B_k_cache, B_v_cache, B_wq, B_wo.T)
        any_spec = pl.BlockSpec(memory_space=pl.ANY)
        outs = pl.pallas_call(
            functools.partial(_kernel, cfg=cfg),
            in_specs=[any_spec] * 11,
            out_specs=[any_spec] * 11,
            out_shape=[sds(grad_out)] + [sds(a) for a in ins],
            scratch_shapes=[
                pltpu.VMEM((2, NR, D), BF),
                pltpu.VMEM((2, NR, DP), BF),
                pltpu.VMEM((2, NR, D), BF),
                pltpu.VMEM((2, NR, DP), BF),
                pltpu.VMEM((2, 2 * DP - D, 128), BF),
                pltpu.VMEM((2, NR // 128, DP - D, 128), BF),
                pltpu.VMEM((2, R, NR // 128, HD, 128), BF),
                pltpu.VMEM((2, R, 2, NR, 128), BF),
                pltpu.VMEM((2, R, HD, NR), F32),
                pltpu.VMEM((2, R, NR, HH), BF),
                pltpu.VMEM((2, 2, R, DH, HH), BF),
                [pltpu.VMEM((2, R, HQ, HH), F32)] * 2,
                [pltpu.VMEM((2, R, HQ, HH), BF)] * 3,
                [pltpu.VMEM((2, R, HK, HH), BF)] * 3,
                [pltpu.VMEM((2, R, HQ, HK), F32)] * 2,
                [pltpu.VMEM((2, R, 2, HQ, 128), BF)] * 2,
                [pltpu.VMEM((2, R, HQ, HH), F32)] * 2,
                [pltpu.VMEM((2, R, HK, HH), F32)] * 2,
                pltpu.VMEM((2, R, HD, HH), F32),
                pltpu.VMEM((2, NB, SK, DH), BF),
                pltpu.VMEM((2, NB, SK, DH), BF),
                pltpu.VMEM((2, 2, NB, SK, HH) if cfg.get('dsplit') else (2, NB, SK, DH), BF),
                pltpu.VMEM((2, 2, NB, SK, HH) if cfg.get('dsplit') else (2, NB, SK, DH), BF),
                pltpu.VMEM((2, D, DH), BF),
                pltpu.VMEM((2, D, DH), BF),
                pltpu.VMEM((2, D, DH), BF),
                pltpu.VMEM((2, D, DH), BF),
                pltpu.SemaphoreType.DMA((4, 2)),
                pltpu.SemaphoreType.DMA((4, 2)),
                pltpu.SemaphoreType.DMA((4,)),
            ],
            compiler_params=pltpu.CompilerParams(
                vmem_limit_bytes=110 * 2 ** 20,
                flags=flags,
            ),
        )(*ins, grad_out)
        return (*outs[:5], outs[5].T, *outs[6:10], outs[10].T)
    return fn


pallas_concat_heads__mha_block_cached__gqa_block_cached__near_ridge_kernel = make(order=7, dsplit=1, zm=1)
```

```python
import functools

import jax
import jax.numpy as jnp
from jax import lax
from jax.experimental import pallas as pl
from jax.experimental.pallas import tpu as pltpu

NB, SQ, D, H, SK, DH = 8, 224, 448, 16, 512, 256
HQ, HD, HK, HH = SQ // 2, D // 2, SK // 2, DH // 2
NR = NB * HQ
LN = 128
NT_ROWS = NR // LN
DF = 3 * LN
DT = D - DF
R = 7
SCALE = DH ** -0.5
BF, F32, U32 = jnp.bfloat16, jnp.float32, jnp.uint32
NN = (((1,), (0,)), ((), ()))
NT = (((1,), (1,)), ((), ()))
TN = (((0,), (0,)), ((), ()))


def _dot(a, b, dims):
    return lax.dot_general(a, b, dims, preferred_element_type=F32)


class _Strassen:
    raw_v = {1: (0, 0), 4: (1, 1)}
    order_u = (0, 4, 5, 3, 2, 1, 6)
    order_v = (0, 1, 3, 5, 2, 6, 4)
    order_w = (0, 3, 4, 6, 1, 2, 5)

    @staticmethod
    def forms_u(a11, a12, a21, a22):
        return [a11 + a22, a21 + a22, a11, a22, a11 + a12, a21 - a11, a12 - a22]

    @staticmethod
    def forms_v(b11, b12, b21, b22):
        return [b11 + b22, b11, b12 - b22, b21 - b11, b22, b11 + b12, b21 + b22]

    @staticmethod
    def forms_w(c11, c12, c21, c22):
        return [c11 + c22, c21 - c22, c12 + c22, c11 + c21, c12 - c11, c22, c11]

    @staticmethod
    def comb_u(d):
        return (d[2] + d[0] + d[4] - d[5], d[4] + d[6], d[1] + d[5], d[1] - d[6] + d[0] + d[3])

    @staticmethod
    def comb_v(d):
        return (d[1] + d[0] - d[3] + d[5], d[2] + d[5], d[3] + d[6], d[6] - d[2] + d[0] + d[4])

    @staticmethod
    def comb_w(m):
        return (m[6] + m[0] + m[3] - m[4], m[2] + m[4], m[1] + m[3], m[5] - m[1] + m[2] + m[0])


class _Winograd:
    raw_v = {0: (0, 0), 1: (1, 0), 2: (1, 1)}
    order_u = (5, 2, 4, 6, 0, 1, 3)
    order_v = (3, 5, 4, 6, 1, 0, 2)
    order_w = (0, 5, 6, 4, 1, 2, 3)

    @staticmethod
    def forms_u(a11, a12, a21, a22):
        s1 = a21 + a22
        s2 = s1 - a11
        return [a11, a12, a12 - s2, a22, s1, s2, a11 - a21]

    @staticmethod
    def forms_v(b11, b12, b21, b22):
        t1 = b12 - b11
        t2 = b22 - t1
        return [b11, b21, b22, b21 - t2, t1, t2, b22 - b12]

    @staticmethod
    def forms_w(c11, c12, c21, c22):
        u3 = c21 + c22
        u2 = u3 + c12
        return [c11 + u2, c11, c12, c21, c12 + c22, u2, u3]

    @staticmethod
    def comb_u(d):
        s2 = d[5] - d[2]
        s1 = d[4] + s2
        return (d[0] + (d[6] - s2), d[1] + d[2], s1 - d[6], d[3] + s1)

    @staticmethod
    def comb_v(d):
        t2 = d[5] - d[3]
        t1 = d[4] - t2
        return (d[0] - t1, t1 - d[6], d[1] + d[3], d[2] + (t2 + d[6]))

    @staticmethod
    def comb_w(m):
        u2 = m[0] + m[5]
        u3 = u2 + m[6]
        return (m[0] + m[1], (u2 + m[4]) + m[2], u3 + m[3], u3 + m[4])


ALG = (_Strassen, _Winograd)
ALG_AW = _Winograd


def _rows(c, n=16):
    return slice(c * n, (c + 1) * n)


def _load_bf16(ref, *idx):
    return pltpu.bitcast(ref.bitcast(U32)[idx], BF)


ORDER = ("P0 P1 S0 P2 P3 Y0 S1 P4 P5 Z0 Y1 S2 P6 P7 Z1 Y2 S3 A0 A1 Z2 Y3 "
         "S4 A2 W03a Z3 Y4 S5 A3 W03b Z4 Y5 S6 W35a A4 Z5 Y6 S7 A5 W35b Z6 Y7 Z7 W57 A6")
SOFTMAX_MARGIN = (530, 750, 750, 700, 650, 650, 780, 750)


def _plan():
    both = lambda rs: [(h, r) for h in range(2) for r in rs]
    seq = dict(
        P=[(h, r) for h in range(2) for r in ALG[h].order_v[:6] + (7, 8, 9) + ALG[h].order_v[6:]],
        S=[(h, r, n) for h in range(2) for n in range(2) for r in ALG[h].order_w],
        Y=[(h, r) for h in range(2) for r in ALG[h].order_u],
        Z=[(h, r) for h in range(2) for r in ALG[h].order_v],
        A=both(range(R)), W=both(range(R)))
    mm = []
    for g in ORDER.split():
        index = tuple(int(ch) for ch in g if ch.isdigit())
        mm += [(g[0],) + index + hr for hr in seq[g[0]] if g[-1].isdigit() or hr[0] == 'ab'.index(g[-1])]

    def cycles(t):
        if t[0] == 'W':
            return 56 * (t[2] - t[1])
        if t[0] == 'P':
            return 28 if t[3] < R else 56
        return dict(S=28, Y=56, Z=64, A=56)[t[0]]

    start, now = {}, 0
    for t in mm:
        start[t] = now
        now += cycles(t)
    pick = lambda *key: [i for i, t in enumerate(mm) if t[:len(key)] == key]
    after = [[] for _ in range(len(mm) + 1)]
    for b in range(NB):
        first_s = pick('S', b)[0]
        for h in range(2):
            after[pick('P', b, h)[-1] + 1] += [('PC', b, h, c) for c in range(7)]
            after[first_s - 14] += [('KV', b, h, c) for c in range(16)]
            after[pick('Y', b, h)[-1] + 1] += [('YC', b, h, c) for c in range(7)]
            after[pick('Z', b, h)[-1] + 1].append(('ZC', b, h))
        last_s, need = pick('S', b)[-1], min(pick('Y', b) + pick('Z', b))
        t0, t1 = start[mm[last_s]] + cycles(mm[last_s]), start[mm[need]] - SOFTMAX_MARGIN[b]
        for c in range(7):
            gates = []
            for c8 in (2 * c, 2 * c + 1):
                later = [i for i in range(last_s + 1, need - 2) if start[mm[i]] >= t0 + (t1 - t0) * c8 / 13.0]
                gates.append(later[0] if c8 and later else last_s)
            after[gates[1] + 1].append(('SM', b, c, [mm[i] if i > last_s else None for i in gates]))
    for h in range(2):
        after[max([i for i, t in enumerate(mm) if t[0] == 'W' and t[3] == h]) + 1].append(('F', h))
        after[0].append(('WA', h))
        after[pick('W')[(14, 21)[h]]].append(('WP', h))
    after[0].insert(0, ('DMA',))
    out = list(after[0])
    for i, t in enumerate(mm):
        out += [t] + after[i + 1]
    return out


def _kernel(ax, ak, av, awq, awo, bx, bk, bv, bwq, bwo, g_hbm,
            out_hbm, dax, dak, dav, dawq, dawo, dbx, dbk, dbv, dbwq, dbwo,
            xin, gin, dxst, ost, tail, xw, xp, acc, wa, wp, uf, vf, wf, vy,
            kvbuf, dkvbuf, wbuf, dwbuf, sem_w, sem_kv, sem_dkv, sem_dw, sem_x):
    n_heads = 2 * H

    def head_cols(h):
        return pl.ds(h * DH if isinstance(h, int) else pl.multiple_of(h * DH, DH), DH)

    def w_copies(br, h, s):
        return [pltpu.make_async_copy(w.at[:, head_cols(h)], wbuf.at[s, i], sem_w.at[s])
                for i, w in enumerate(((awq, awo), (bwq, bwo))[br])]

    def kv_copies(br, h, s):
        return [pltpu.make_async_copy(c.at[:, h, :, pl.ds(k * HH, HH)], kvbuf.at[s, i, k], sem_kv.at[s])
                for i, c in enumerate(((ak, av), (bk, bv))[br]) for k in range(2)]

    def dkv_copies(br, h, s):
        return [pltpu.make_async_copy(dkvbuf.at[s, i, k], c.at[:, h, :, pl.ds(k * HH, HH)], sem_dkv.at[s])
                for i, c in enumerate(((dak, dav), (dbk, dbv))[br]) for k in range(2)]

    def dw_copies(br, h, s):
        return [pltpu.make_async_copy(dwbuf.at[s, i], w.at[:, head_cols(h)], sem_dw.at[s])
                for i, w in enumerate(((dawq, dawo), (dbwq, dbwo))[br])]

    def grad_copies(br, h, s):
        return dkv_copies(br, h, s) + dw_copies(br, h, s)

    def start_for(copies, t, s):
        @pl.when(t < H)
        def _():
            for c in copies(0, jnp.minimum(t, H - 1), s):
                c.start()

        @pl.when(t >= H)
        def _():
            for c in copies(1, jnp.clip(t - H, 0, H - 1), s):
                c.start()

    def wait(copies):
        for c in copies:
            c.wait()

    def wait_all(buf, sem):
        pltpu.make_async_copy(buf, buf, sem).wait()

    def by_row_half(hbm, vm, sem, lanes=None, vm_lanes=None, store=False):
        cs = []
        for b in range(NB):
            for j in range(2):
                h_ = hbm.at[b, pl.ds(j * HQ, HQ)] if lanes is None else hbm.at[b, pl.ds(j * HQ, HQ), lanes]
                v_ = vm.at[j, pl.ds(b * HQ, HQ)] if lanes is None else vm.at[j, pl.ds(b * HQ, HQ), vm_lanes]
                cs.append(pltpu.make_async_copy(v_, h_, sem) if store else pltpu.make_async_copy(h_, v_, sem))
        return cs

    full, shared = pl.ds(0, DF), pl.ds(DF, LN)
    x_in = [by_row_half(ax, xin, sem_x.at[0]) + by_row_half(g_hbm, gin, sem_x.at[0], pl.ds(0, DF + LN), pl.ds(0, DF + LN)),
            by_row_half(bx, xin, sem_x.at[0]) + by_row_half(g_hbm, gin, sem_x.at[0], pl.ds(DF + LN, DF), full)]
    x_out = [by_row_half(dax, dxst, sem_x.at[1], store=True) + by_row_half(out_hbm, ost, sem_x.at[1], full, full, True),
             by_row_half(dbx, dxst, sem_x.at[1], store=True)
             + by_row_half(out_hbm, ost, sem_x.at[1], pl.ds(DF + LN, DF), full, True)
             + by_row_half(out_hbm, ost, sem_x.at[1], shared, shared, True)]

    def a_weight_forms(s, half):
        w = wbuf[s, half].astype(F32)
        if half == 0:
            w = w * SCALE
        for r, f in enumerate(ALG_AW.forms_u(w[:HD, :HH], w[:HD, HH:], w[HD:, :HH], w[HD:, HH:])):
            wa[half, r] = f.astype(BF)

    def p_weight_forms(s, half, br):
        if half == 0:
            wd, w3 = wbuf[s, half, :DF, :].astype(F32) * SCALE, wbuf[s, half, DF:, :].astype(F32) * SCALE
        else:
            wd = wbuf[s, half, pl.ds(pl.multiple_of(br * DT, DT), DF), :].astype(F32)
            w3 = wbuf[s, half, pl.ds(pl.multiple_of((1 - br) * DF, DT), DT), :].astype(F32)
        w1, w2 = wd[2 * LN:2 * LN + DT], wd[2 * LN + DT:]
        fs = ALG[half].forms_u(wd[:LN, :HH], wd[:LN, HH:], wd[LN:2 * LN, :HH], wd[LN:2 * LN, HH:]) + [
            jnp.concatenate([w1[:, :HH], w2[:, :HH] - w2[:, HH:]], axis=0),
            jnp.concatenate([w1[:, HH:], w3[:, HH:] - w3[:, :HH]], axis=0),
            jnp.concatenate([w3[:, :HH], w2[:, HH:]], axis=0)]
        for r, f in enumerate(fs):
            wp[half, r] = f.astype(BF)

    def input_forms(br, n, carry):
        rr = pl.ds(pl.multiple_of(n * LN, LN), LN)
        low = lax.broadcasted_iota(jnp.int32, (LN, LN), 1) < DT
        for half, src in enumerate((xin, gin)):
            x = [src[j, rr, :].astype(F32) for j in range(2)]
            for r, f in enumerate(ALG[half].forms_w(x[0][:, :LN], x[1][:, :LN], x[0][:, LN:2 * LN], x[1][:, LN:2 * LN])):
                xp[half, r, rr, :] = f.astype(BF)
            ts = []
            for j in range(2):
                s12, s3 = x[j][:, 2 * LN:DF], x[j][:, DF:]
                if half == 0:
                    s3 = jnp.concatenate([s3, s3], axis=1)
                else:
                    s3 = jnp.where(low if br == 0 else ~low, s3, pltpu.roll(s3, DT, 1))
                for k, f in enumerate((s12, jnp.where(low, s12, s3), jnp.where(low, s3, s12))):
                    xp[half, R + 2 * k + j, rr, :] = f.astype(BF)
                whole, rest = x[j][:, :DF].T, s3.T[:DT]
                ts.append(jnp.concatenate([rest, whole] if half == 1 and br == 1 else [whole, rest], axis=0))
            for r, f in enumerate(ALG_AW.forms_w(ts[0][:HD], ts[1][:HD], ts[0][HD:], ts[1][HD:])):
                xw[half, r, n] = f.astype(BF)
        return carry

    def finish(br, n, carry):
        rr = pl.ds(pl.multiple_of(n * LN, LN), LN)
        for half in range(2):
            c11, c12, c21, c22 = ALG_AW.comb_w([acc[br, half, r, n] for r in range(R)])
            for j, (top, bot) in enumerate(((c11, c21), (c12, c22))):
                y = jnp.concatenate([top, bot], axis=0)
                if half == 0:
                    dxst[j, rr, :DF] = y[:DF].T.astype(BF)
                    dxst[j, rr, DF:] = jnp.concatenate([y[DF:], y[DF:]], axis=0).T[:, :DT].astype(BF)
                elif br == 0:
                    ost[j, rr, :DF] = y[:DF].T.astype(BF)
                    tail[j, n] = y[DF:]
                else:
                    ost[j, rr, :DF] = y[DT:].T.astype(BF)
                    ost[j, rr, DF:] = jnp.concatenate([tail[j, n], y[:DT]], axis=0).T.astype(BF)
        return carry

    def head(t, carry):
        slot = t % 2
        br = t // H
        never = t < 0
        val, paced_by = {}, {}

        def start_copies():
            @pl.when(t + 1 < n_heads)
            def _():
                start_for(kv_copies, t + 1, 1 - slot)
                start_for(w_copies, t + 2, (t + 2) % 3)

            @pl.when(t > 0)
            def _():
                start_for(grad_copies, jnp.maximum(t - 1, 0), 1 - slot)

        wait_all(kvbuf.at[slot], sem_kv.at[slot])
        wait_all(wbuf.at[(t + 1) % 3], sem_w.at[(t + 1) % 3])

        @pl.when(t >= 2)
        def _():
            wait_all(dkvbuf.at[slot], sem_dkv.at[slot])
            wait_all(dwbuf.at[slot], sem_dw.at[slot])

        def p_mm(b, half, r):
            rr = _rows(b, HQ // 2)
            if r < R:
                lhs = _load_bf16(xp, half, r, rr)
            else:
                lhs = jnp.concatenate([_load_bf16(xp, half, R + 2 * (r - R) + j, rr) for j in range(2)], axis=0)
            val['p', b, half, r] = _dot(lhs, _load_bf16(wp, half, r), NN)
            return val['p', b, half, r]

        def p_comb(b, half, c):
            blocks = ALG[half].comb_v([val['p', b, half, r][_rows(c)] for r in range(R)])
            rest = lambda r, j: val['p', b, half, r][_rows(j * 7 + c)]
            t11, t12, t21, t22 = [blk + (rest(R + k, j) + rest(R + 2, j))
                                  for blk, (k, j) in zip(blocks, ((0, 0), (0, 1), (1, 0), (1, 1)))]
            for r, f in enumerate(ALG[half].forms_u(t11, t21, t12, t22)):
                uf[b][half, r, _rows(c), :] = f.astype(BF)

        def kv_forms(b, half, c):
            raw = [_load_bf16(kvbuf, slot, half, k, b, _rows(j * 16 + c, 8)).astype(F32)
                   for k, j in ((0, 0), (0, 1), (1, 0), (1, 1))]
            for r, f in enumerate(ALG[half].forms_v(*raw)):
                if r not in ALG[half].raw_v:
                    vf[b][half, r, _rows(c), :] = f.astype(BF)

        def v_form(b, half, r, lo=0, n=HK):
            if r in ALG[half].raw_v:
                k, j = ALG[half].raw_v[r]
                return _load_bf16(kvbuf, slot, half, k, b, pl.ds((j * HK + lo) // 2, n // 2))
            return _load_bf16(vf[b], half, r, pl.ds(lo // 2, n // 2))

        def s_mm(b, half, r, n):
            val['s', b, half, r, n] = _dot(_load_bf16(uf[b], half, r), v_form(b, half, r, n * LN, LN), NT)
            return val['s', b, half, r, n]

        def softmax(b, c, gates):
            def quadrants(half, c8):
                return ALG[half].comb_w([jnp.concatenate([val['s', b, half, r, n][_rows(c8, 8)] for n in range(2)], axis=1)
                               for r in range(R)])

            def put(half, parts):
                quads = [jnp.concatenate([parts[0][i], parts[1][i]], axis=0) for i in range(4)]
                for r, f in enumerate(ALG[half].forms_w(*quads)):
                    for n in range(2):
                        wf[b][half, r, n, _rows(c), :] = f[:, _rows(n, LN)].astype(BF)

            ps = []
            for c8, gate in zip((2 * c, 2 * c + 1), gates):
                s11, s12, s21, s22 = quadrants(0, c8)
                p4 = []
                for sa, sb in ((s11, s12), (s21, s22)):
                    mx = jnp.maximum(sa, sb)
                    mx = jnp.maximum(mx[:, :LN], mx[:, LN:])
                    if gate is not None:
                        mx = jnp.where(never, paced_by[gate], mx)
                    m = jnp.max(mx, axis=-1, keepdims=True)
                    ea, eb = jnp.exp(sa - m), jnp.exp(sb - m)
                    l = jnp.sum(ea + eb, axis=-1, keepdims=True)
                    inv = pl.reciprocal(l, approx=True)
                    inv = inv * (2.0 - l * inv)
                    p4 += [ea * inv, eb * inv]
                ps.append(p4)
            put(1, ps)
            dss = []
            for p4, c8 in zip(ps, (2 * c, 2 * c + 1)):
                d4 = quadrants(1, c8)
                ds4 = []
                for i in (0, 2):
                    delta = jnp.sum(p4[i] * d4[i] + p4[i + 1] * d4[i + 1], axis=-1, keepdims=True)
                    ds4 += [p4[i] * (d4[i] - delta), p4[i + 1] * (d4[i + 1] - delta)]
                dss.append(ds4)
            put(0, dss)

        def w_form(b, half, r):
            return jnp.concatenate([_load_bf16(wf[b], half, r, n) for n in range(2)], axis=1)

        def y_mm(b, half, r):
            val['y', b, half, r] = _dot(w_form(b, half, r), v_form(b, half, r), NN)
            return val['y', b, half, r]

        def y_comb(b, half, c):
            y11, y12, y21, y22 = ALG[half].comb_u([val['y', b, half, r][_rows(c)] for r in range(R)])
            for r, f in enumerate(ALG_AW.forms_v(y11, y21, y12, y22)):
                vy[half, r, _rows(b * 7 + c), :] = f.astype(BF)

        def z_mm(b, half, r):
            val['z', b, half, r] = _dot(w_form(b, half, r), _load_bf16(uf[b], half, r), TN)
            return val['z', b, half, r]

        def z_comb(b, half):
            z = ALG[half].comb_v([val['z', b, half, r] for r in range(R)])
            for (k, j), zz in zip(((0, 0), (0, 1), (1, 0), (1, 1)), z):
                dkvbuf[slot, half, k, b, _rows(j, HK), :] = zz.astype(BF)

        def a_mm(n, half, r):
            d = _dot(_load_bf16(wa, half, r), _load_bf16(vy, half, r, _rows(n, LN // 2)), NT)
            acc[br, half, r, n] += d
            return d

        def w_mm(lo, hi, half, r):
            lhs = jnp.concatenate([_load_bf16(xw, half, r, n) for n in range(lo, hi)], axis=1)
            d = _dot(lhs, _load_bf16(vy, half, r, slice(lo * LN // 2, hi * LN // 2)), NN)
            val['d', half, r] = d if lo == 0 else val['d', half, r] + d
            return d

        def w_comb(half):
            a11, a12, a21, a22 = ALG_AW.comb_u([val['d', half, r] for r in range(R)])
            dw = jnp.concatenate([jnp.concatenate([a11, a12], axis=1), jnp.concatenate([a21, a22], axis=1)], axis=0)
            dwbuf[slot, half] = (dw * SCALE if half == 0 else dw).astype(BF)

        tasks = dict(P=p_mm, PC=p_comb, KV=kv_forms, S=s_mm, SM=softmax, Y=y_mm, YC=y_comb, Z=z_mm, ZC=z_comb,
                     A=a_mm, W=w_mm, F=w_comb, DMA=start_copies,
                     WA=lambda half: a_weight_forms(t % 3, half),
                     WP=lambda half: p_weight_forms((t + 1) % 3, half, jnp.minimum((t + 1) // H, 1)))
        for task in _plan():
            res = tasks[task[0]](*task[1:])
            if res is not None:
                paced_by[task] = res[:8, :LN]

        return carry

    def switch_branch(n, carry):
        finish(0, n, carry)
        return input_forms(1, n, carry)

    def branch(br, carry):
        lax.fori_loop(br * H, (br + 1) * H, head, 0)

        @pl.when(br == 0)
        def _():
            wait(x_in[1])
            lax.fori_loop(0, NT_ROWS, switch_branch, 0)
            for c in x_out[0]:
                c.start()
        return carry

    def zero_acc(i, carry):
        acc[i // (2 * R), (i // R) % 2, i % R] = jnp.zeros((NT_ROWS, HD, LN), F32)
        return carry

    for c in w_copies(0, 0, 0) + x_in[0]:
        c.start()
    lax.fori_loop(0, 4 * R, zero_acc, 0)
    wait(w_copies(0, 0, 0))
    for c in kv_copies(0, 0, 0) + w_copies(0, 1, 1):
        c.start()
    for half in range(2):
        p_weight_forms(0, half, jnp.int32(0))
    wait(x_in[0])
    lax.fori_loop(0, NT_ROWS, functools.partial(input_forms, 0), 0)
    for c in x_in[1]:
        c.start()
    lax.fori_loop(0, 2, branch, 0)
    for c in grad_copies(1, H - 1, 1):
        c.start()
    wait(x_out[0])
    lax.fori_loop(0, NT_ROWS, functools.partial(finish, 1), 0)
    for c in x_out[1]:
        c.start()
    for s in range(2):
        wait_all(dkvbuf.at[s], sem_dkv.at[s])
        wait_all(dwbuf.at[s], sem_dw.at[s])
    wait(x_out[1])


@jax.jit
def pallas_concat_heads__mha_block_cached__gqa_block_cached__near_ridge_kernel(
        A_x, A_k_cache, A_v_cache, A_wq, A_wo, B_x, B_k_cache, B_v_cache, B_wq, B_wo, grad_out):
    ins = (A_x, A_k_cache, A_v_cache, A_wq, A_wo.T, B_x, B_k_cache, B_v_cache, B_wq, B_wo.T)
    hbm = pl.BlockSpec(memory_space=pl.ANY)
    outs = pl.pallas_call(
        _kernel,
        in_specs=[hbm] * 11,
        out_specs=[hbm] * 11,
        out_shape=[jax.ShapeDtypeStruct(a.shape, BF) for a in (grad_out,) + ins],
        scratch_shapes=[
            pltpu.VMEM((2, NR, D), BF),
            pltpu.VMEM((2, NR, DF + LN), BF),
            pltpu.VMEM((2, NR, D), BF),
            pltpu.VMEM((2, NR, DF + LN), BF),
            pltpu.VMEM((2, NT_ROWS, DT, LN), F32),
            pltpu.VMEM((2, R, NT_ROWS, HD, LN), BF),
            pltpu.VMEM((2, R + 6, NR, LN), BF),
            pltpu.VMEM((2, 2, R, NT_ROWS, HD, LN), F32),
            pltpu.VMEM((2, R, HD, HH), BF),
            pltpu.VMEM((2, R + 3, LN, HH), BF),
            [pltpu.VMEM((2, R, HQ, HH), BF)] * NB,
            [pltpu.VMEM((2, R, HK, HH), BF)] * NB,
            [pltpu.VMEM((2, R, 2, HQ, LN), BF)] * NB,
            pltpu.VMEM((2, R, NR, HH), BF),
            pltpu.VMEM((2, 2, 2, NB, SK, HH), BF),
            pltpu.VMEM((2, 2, 2, NB, SK, HH), BF),
            pltpu.VMEM((3, 2, D, DH), BF),
            pltpu.VMEM((2, 2, D, DH), BF),
            pltpu.SemaphoreType.DMA((3,)),
            pltpu.SemaphoreType.DMA((2,)),
            pltpu.SemaphoreType.DMA((2,)),
            pltpu.SemaphoreType.DMA((2,)),
            pltpu.SemaphoreType.DMA((2,)),
        ],
        compiler_params=pltpu.CompilerParams(
            vmem_limit_bytes=110 * 2 ** 20,
            disable_bounds_checks=True,
            flags={"XLA_TPU_FORCE_LP_LLO_SCHEDULER": True, "XLA_TPU_MAX_INSTS_TO_PREDICATE": 32},
        ),
    )(*ins, grad_out)
    return (*outs[:5], outs[5].T, *outs[6:10], outs[10].T)
```
